```python
import jax
import jax.numpy as jnp

def _softmax(x, axis=-1):
    return jax.nn.softmax(x, axis=axis)
def _gelu(x):
    return jax.nn.gelu(x, approximate=True)
def _silu(x):
    return jax.nn.silu(x)
def _sigmoid(x):
    return jax.nn.sigmoid(x)
def _layernorm(x, axis=-1, eps=1e-5):
    m = jnp.mean(x, axis=axis, keepdims=True)
    v = jnp.var(x, axis=axis, keepdims=True)
    return (x - m) / jnp.sqrt(v + eps)
def _scatter_add(tgt, idx, src, axis=0):
    return tgt.at[idx].add(src)
def _segment_sum(src, seg, n):
    return jax.ops.segment_sum(src, seg, n)
class _Rng:
    def __init__(self, key):
        self._k = key
    def _next(self):
        self._k, sub = jax.random.split(self._k)
        return sub
    def normal(self, shape):
        return jax.random.normal(self._next(), shape, dtype=jnp.bfloat16)
    def randint(self, lo, hi, shape):
        return jax.random.randint(self._next(), shape, lo, hi, dtype=jnp.int32)
    def uniform(self, shape, lo=0.0, hi=1.0):
        return jax.random.uniform(self._next(), shape, jnp.bfloat16, lo, hi)
    def permutation(self, n):
        return jax.random.permutation(self._next(), n)


kernel_name = 'parallel_sum__sliding_block_cached__glu_gated_swiglu__decode'

def setup_inputs():
    _rng = _Rng(jax.random.key(int.from_bytes(__import__("os").urandom(4), "little")))
    _w = (lambda a: (lambda t: t.astype(jnp.bfloat16) if jnp.issubdtype(t.dtype, jnp.floating) else t)(jnp.asarray(a)))
    def _A_setup():
        B, Sq, D = 4, 1, 640
        Hq, Hkv, Sk, Dh = 32, 32, 8192, 192
        assert Hq % Hkv == 0, (Hq, Hkv)
        return {
            "x": _w((lambda *s: _rng.normal(s) * 0.05)(B, Sq, D)),
            "k_cache": _w((lambda *s: _rng.normal(s) * 0.05)(B, Hkv, Sk, Dh)),
            "v_cache": _w((lambda *s: _rng.normal(s) * 0.05)(B, Hkv, Sk, Dh)),
            "wq": _w((lambda *s: _rng.normal(s) * 0.05)(D, Hq * Dh) * (D ** -0.5)),
            "wo": _w((lambda *s: _rng.normal(s) * 0.05)(Hq * Dh, D) * ((Hq * Dh) ** -0.5)),
        }
    _A_in = _A_setup()

    def _B_setup():
        B, S, D, F = 4, 1, 640, 1536
        return {
            "x": _w((lambda *s: _rng.normal(s) * 0.05)(B, S, D)),
            "w1": _w((lambda *s: _rng.normal(s) * 0.05)(D, F) * (2.0 / D) ** 0.5),
            "w3": _w((lambda *s: _rng.normal(s) * 0.05)(D, F) * (2.0 / D) ** 0.5),
            "w2": _w((lambda *s: _rng.normal(s) * 0.05)(F, D) * (2.0 / F) ** 0.5),
        }
    _B_in = _B_setup()

    return {
        "A_x": _A_in["x"],
        "A_k_cache": _A_in["k_cache"],
        "A_v_cache": _A_in["v_cache"],
        "A_wq": _A_in["wq"],
        "A_wo": _A_in["wo"],
        "B_x": _B_in["x"],
        "B_w1": _B_in["w1"],
        "B_w3": _B_in["w3"],
        "B_w2": _B_in["w2"],
    }

def reference(A_x, A_k_cache, A_v_cache, A_wq, A_wo, B_x, B_w1, B_w3, B_w2):
    def _A_ref(x, k_cache, v_cache, wq, wo):
        B, Sq, D = x.shape
        Hq, Dh = 32, 192
        Hkv, Sk = k_cache.shape[1], k_cache.shape[2]
        W = min(4096, max(256, Sk // 4))
        rep = Hq // Hkv
        q = (lambda x, *d: x.transpose(*d))((x @ wq).reshape(B, Sq, Hq, Dh), 0, 2, 1, 3)
        k = jnp.repeat(k_cache[:, :, Sk - W:, :], rep, axis=1)
        v = jnp.repeat(v_cache[:, :, Sk - W:, :], rep, axis=1)
        scores = jnp.einsum("bhqd,bhkd->bhqk", q, k) * (Dh ** -0.5)
        p = _softmax(scores, axis=-1)
        o = jnp.einsum("bhqk,bhkd->bhqd", p, v)
        return (lambda x, *d: x.transpose(*d))(o, 0, 2, 1, 3).reshape(B, Sq, Hq * Dh) @ wo

    def _B_ref(x, w1, w3, w2):
        gate = jnp.einsum("bsd,df->bsf", x, w1)
        up = jnp.einsum("bsd,df->bsf", x, w3)
        h = _silu(gate) * up
        out = jnp.einsum("bsf,fd->bsd", h, w2)
        return out

    x = A_x
    xn = _layernorm(x, axis=-1)
    return x + _A_ref(xn, A_k_cache, A_v_cache, A_wq, A_wo) + _B_ref(xn, B_w1, B_w3, B_w2)
```

```python
import jax
import jax.numpy as jnp
import jax.experimental.pallas as pl
import jax.experimental.pallas.tpu as pltpu

B, D, H, DH, F = 4, 640, 32, 192, 1536

RK, RV = 2, 2
FFN_AT = 6
CS, NF = 2, 4

def _kernel(x_hbm, kt_hbm, vt_hbm, wq_hbm, wo_hbm, w1_hbm, w3_hbm, w2_hbm, o_ref,
           xb, kb, vb, wqb, wob, w1b, w3b, w2b, q_scr, p_scr, ksem, vsem, tsem, wsem):
    SK = kt_hbm.shape[3]
    W = min(4096, max(256, SK // 4))
    CW = W // CS
    L = H - 1
    def kc(h, slot):
        return pltpu.make_async_copy(kt_hbm.at[:, h, :, pl.ds(SK - W, W)], kb.at[slot], ksem.at[slot])
    def vc(h, slot):
        return pltpu.make_async_copy(vt_hbm.at[:, h, :, pl.ds(SK - W, W)], vb.at[slot], vsem.at[slot])
    chunks = [(b, c) for b in range(B) for c in range(CS)]
    def tc(i):
        b, c = chunks[i]
        return pltpu.make_async_copy(vt_hbm.at[b, L, :, pl.ds(SK - W + c * CW, CW)],
                                     vb.at[L % RV, b, :, pl.ds(c * CW, CW)], tsem.at[i])
    xc = pltpu.make_async_copy(x_hbm, xb, wsem.at[0])
    wqc = pltpu.make_async_copy(wq_hbm, wqb, wsem.at[1])
    woc = pltpu.make_async_copy(wo_hbm, wob, wsem.at[2])
    w1c = pltpu.make_async_copy(w1_hbm, w1b, wsem.at[3])
    w3c = pltpu.make_async_copy(w3_hbm, w3b, wsem.at[4])
    w2c = pltpu.make_async_copy(w2_hbm, w2b, wsem.at[5])
    wqc.start(); xc.start()
    for i in range(max(RK, RV)):
        if i < RK: kc(i, i).start()
        if i < RV: vc(i, i).start()
        if i == 0: woc.start()
    w1c.start(); w3c.start(); w2c.start()
    xc.wait()
    x = xb[0].astype(jnp.float32)
    m = jnp.mean(x, axis=-1, keepdims=True)
    xm = x - m
    v = jnp.mean(xm * xm, axis=-1, keepdims=True)
    xn = (xm / jnp.sqrt(v + 1e-5))
    xn8 = jnp.concatenate([xn, jnp.zeros_like(xn)], axis=0).astype(jnp.bfloat16)
    wqc.wait()
    q = jnp.dot(xn8, wqb[...], preferred_element_type=jnp.float32)
    row = jax.lax.broadcasted_iota(jnp.int32, (8, B * DH), 0)
    col = jax.lax.broadcasted_iota(jnp.int32, (8, B * DH), 1) // DH
    for h in range(H):
        qh = q[:, h * DH:(h + 1) * DH]
        q_scr[h] = jnp.where(row == col, jnp.concatenate([qh] * B, axis=1), 0.0)

    def scores(h):
        slot = h % RK
        kc(h, slot).wait()
        qd = q_scr[h].astype(jnp.bfloat16)
        s = jnp.dot(qd, kb[slot].reshape(B * DH, W), preferred_element_type=jnp.float32) * (DH ** -0.5)
        @pl.when(h + RK < H)
        def _():
            kc(h + RK, slot).start()
        mx = jnp.max(s, axis=-1, keepdims=True)
        e = jnp.exp(s - mx)
        p_scr[...] = e / jnp.sum(e, axis=-1, keepdims=True)

    r = jax.lax.broadcasted_iota(jnp.int32, (8, DH), 0)
    def wo_dot(o, h):
        off = h * DH if isinstance(h, int) else pl.multiple_of(h * DH, DH)
        return jnp.dot(o.astype(jnp.bfloat16), wob[pl.ds(off, DH), :], preferred_element_type=jnp.float32)
    NT = (((1,), (1,)), ((), ()))
    def body(h, acc):
        slot = h % RV
        vc(h, slot).wait()
        O = jax.lax.dot_general(p_scr[...].astype(jnp.bfloat16), vb[slot].reshape(B * DH, W), NT, preferred_element_type=jnp.float32)
        @pl.when(h + RV < L)
        def _():
            vc(h + RV, slot).start()
        @pl.when(h + RV == L)
        def _():
            for i in range(NF): tc(i).start()
        o = jnp.zeros((8, DH), jnp.float32)
        for b in range(B):
            o = jnp.where(r == b, O[:, b * DH:(b + 1) * DH], o)
        acc = acc + wo_dot(o, h)
        scores(h + 1)
        return acc

    scores(0)
    woc.wait()
    acc = jnp.zeros((8, D), jnp.float32)
    acc = jax.lax.fori_loop(0, FFN_AT, body, acc)
    w1c.wait(); w3c.wait(); w2c.wait()
    g = jnp.dot(xn8, w1b[...], preferred_element_type=jnp.float32)
    u = jnp.dot(xn8, w3b[...], preferred_element_type=jnp.float32)
    hh = (g * jax.nn.sigmoid(g) * u).astype(jnp.bfloat16)
    acc = acc + jnp.dot(hh, w2b[...], preferred_element_type=jnp.float32)
    acc = acc + jnp.concatenate([x, jnp.zeros_like(x)], axis=0)
    acc = jax.lax.fori_loop(FFN_AT, L, body, acc)
    o = jnp.zeros((8, DH), jnp.float32)
    for i, (b, c) in enumerate(chunks):
        tc(i).wait()
        if i + NF < len(chunks): tc(i + NF).start()
        pc = p_scr[:, c * CW:(c + 1) * CW].astype(jnp.bfloat16)
        O = jax.lax.dot_general(pc, vb[L % RV, b, :, c * CW:(c + 1) * CW], NT, preferred_element_type=jnp.float32)
        o = o + jnp.where(r == b, O, 0.0)
    acc = acc + wo_dot(o, L)
    o_ref[0] = acc[:B].astype(o_ref.dtype)

@jax.jit
def pallas_parallel_sum__sliding_block_cached__glu_gated_swiglu__decode_kernel(A_x, A_k_cache, A_v_cache, A_wq, A_wo, B_x, B_w1, B_w3, B_w2):
    SK = A_k_cache.shape[2]
    W = min(4096, max(256, SK // 4))
    kt = jnp.swapaxes(A_k_cache, 2, 3)
    vt = jnp.swapaxes(A_v_cache, 2, 3)
    x = jnp.swapaxes(A_x, 0, 1)
    bf = jnp.bfloat16
    anyspec = pl.BlockSpec(memory_space=pl.ANY)
    out = pl.pallas_call(
        _kernel,
        in_specs=[anyspec] * 8,
        out_specs=pl.BlockSpec(memory_space=pltpu.VMEM),
        out_shape=jax.ShapeDtypeStruct((1, B, D), bf),
        scratch_shapes=[
            pltpu.VMEM((1, B, D), bf),
            pltpu.VMEM((RK, B, DH, W), bf), pltpu.VMEM((RV, B, DH, W), bf),
            pltpu.VMEM((D, H * DH), bf), pltpu.VMEM((H * DH, D), bf),
            pltpu.VMEM((D, F), bf), pltpu.VMEM((D, F), bf), pltpu.VMEM((F, D), bf),
            pltpu.VMEM((H, 8, B * DH), jnp.float32), pltpu.VMEM((8, W), jnp.float32),
            pltpu.SemaphoreType.DMA((RK,)), pltpu.SemaphoreType.DMA((RV,)), pltpu.SemaphoreType.DMA((B * CS,)), pltpu.SemaphoreType.DMA((6,)),
        ],
        compiler_params=pltpu.CompilerParams(vmem_limit_bytes=100 * 1024 * 1024),
    )(x, kt, vt, A_wq, A_wo, B_w1, B_w3, B_w2)
    return jnp.swapaxes(out, 0, 1)
```
